```python
import jax
import jax.numpy as jnp

def _softmax(x, axis=-1):
    return jax.nn.softmax(x, axis=axis)
def _gelu(x):
    return jax.nn.gelu(x, approximate=True)
def _silu(x):
    return jax.nn.silu(x)
def _sigmoid(x):
    return jax.nn.sigmoid(x)
def _layernorm(x, axis=-1, eps=1e-5):
    m = jnp.mean(x, axis=axis, keepdims=True)
    v = jnp.var(x, axis=axis, keepdims=True)
    return (x - m) / jnp.sqrt(v + eps)
def _scatter_add(tgt, idx, src, axis=0):
    return tgt.at[idx].add(src)
def _segment_sum(src, seg, n):
    return jax.ops.segment_sum(src, seg, n)
class _Rng:
    def __init__(self, key):
        self._k = key
    def _next(self):
        self._k, sub = jax.random.split(self._k)
        return sub
    def normal(self, shape):
        return jax.random.normal(self._next(), shape, dtype=jnp.bfloat16)
    def randint(self, lo, hi, shape):
        return jax.random.randint(self._next(), shape, lo, hi, dtype=jnp.int32)
    def uniform(self, shape, lo=0.0, hi=1.0):
        return jax.random.uniform(self._next(), shape, jnp.bfloat16, lo, hi)
    def permutation(self, n):
        return jax.random.permutation(self._next(), n)


kernel_name = 'standalone__instancenorm__prompt'

def setup_inputs():
    _rng = _Rng(jax.random.key(int.from_bytes(__import__("os").urandom(4), "little")))
    _w = (lambda a: (lambda t: t.astype(jnp.bfloat16) if jnp.issubdtype(t.dtype, jnp.floating) else t)(jnp.asarray(a)))
    B, C, H, W = 2, 1024, 2048, 32
    return {
        "x": _w((lambda *s: _rng.normal(s) * 0.05)(B, C, H, W)),
        "g": _w((lambda *s: _rng.normal(s) * 0.05)(C) + 1.0),
        "b": _w((lambda *s: _rng.normal(s) * 0.05)(C)),
    }

def reference(x, g, b):
    mu = x.mean(axis=(-2, -1), keepdims=True)
    var = ((x - mu) * (x - mu)).mean(axis=(-2, -1), keepdims=True)
    xhat = (x - mu) / jnp.sqrt(var + 1e-5)
    return xhat * g.reshape(1, -1, 1, 1) + b.reshape(1, -1, 1, 1)
```

```python
import jax
import jax.numpy as jnp
from jax import lax
import jax.experimental.pallas as pl
import jax.experimental.pallas.tpu as pltpu

_EPS = 1e-5


@jax.jit
def pallas_standalone__instancenorm__prompt_kernel(
    x: jax.Array,
    g: jax.Array,
    b: jax.Array,
):
    B, C, H, W = x.shape
    N = B * C
    S8 = 8
    R = W // S8
    M, J = 16, 8
    G = N // (M * J)
    nsub = G * J
    chunks = (44, 42, 42)
    assert sum(chunks) == nsub
    nslot = max(chunks)
    nacc = 4
    inv_n = 1.0 / (H * W)

    def kernel(g_ref, b_ref, x_hbm, o_hbm, buf, acc_ref, mu_ref, rsem, wsem):
        def rd(sub, slot):
            return pltpu.make_async_copy(
                x_hbm.at[sub // J, :, sub % J], buf.at[slot], rsem.at[slot])

        def wr(sub, slot, r):
            return pltpu.make_async_copy(
                buf.at[slot, :, r], o_hbm.at[sub // J, :, sub % J, r], wsem.at[slot])

        def start_reads(base, n):
            def body(k, c):
                rd(base + k, k).start()
                return c
            lax.fori_loop(0, n, body, 0)

        def start_write(sub, slot):
            for r in range(R):
                wr(sub, slot, r).start()

        def wait_write(sub, slot):
            for r in range(R):
                wr(sub, slot, r).wait()

        def tree(vals):
            while len(vals) > 1:
                vals = [vals[i] + vals[i + 1] for i in range(0, len(vals), 2)]
            return vals[0]

        def allreduce(a):
            a = jnp.sum(a, axis=2, keepdims=True)
            return jnp.sum(a, axis=1, keepdims=True)

        def compute(sub, slot):
            def p1(m, c):
                accs = [None] * nacc
                k = 0
                for r in range(R):
                    for q in range(H // 256):
                        xf = buf[slot, m, r, :, q * 256:(q + 1) * 256].astype(jnp.float32)
                        for h in range(2):
                            v = xf[:, h * 128:(h + 1) * 128]
                            accs[k % nacc] = v if accs[k % nacc] is None else accs[k % nacc] + v
                            k += 1
                acc_ref[m] = tree(accs)
                return c
            lax.fori_loop(0, M, p1, 0)
            mu = allreduce(acc_ref[...]) * inv_n
            mu_ref[...] = jnp.broadcast_to(mu, (M, 8, 128))

            def p2(m, c):
                mu_m = mu_ref[m]
                accs = [None] * nacc
                k = 0
                for r in range(R):
                    for q in range(H // 256):
                        xf = buf[slot, m, r, :, q * 256:(q + 1) * 256].astype(jnp.float32)
                        for h in range(2):
                            d = xf[:, h * 128:(h + 1) * 128] - mu_m
                            v = d * d
                            accs[k % nacc] = v if accs[k % nacc] is None else accs[k % nacc] + v
                            k += 1
                acc_ref[m] = tree(accs)
                return c
            lax.fori_loop(0, M, p2, 0)
            var = allreduce(acc_ref[...]) * inv_n
            rstd = lax.rsqrt(var + _EPS)
            acc_ref[...] = jnp.broadcast_to(rstd, (M, 8, 128))

            inst0 = (sub // J) * (M * J) + sub % J

            def p3(m, c):
                ch = (inst0 + m * J) % C
                s = acc_ref[m] * g_ref[ch]
                t = b_ref[ch] - mu_ref[m] * s
                s2 = jnp.concatenate([s, s], axis=1)
                t2 = jnp.concatenate([t, t], axis=1)
                for r in range(R):
                    for q in range(H // 256):
                        xf = buf[slot, m, r, :, q * 256:(q + 1) * 256].astype(jnp.float32)
                        buf[slot, m, r, :, q * 256:(q + 1) * 256] = (xf * s2 + t2).astype(jnp.bfloat16)
                return c
            lax.fori_loop(0, M, p3, 0)

        start_reads(0, chunks[0])
        base = 0
        for p, n in enumerate(chunks):
            def body(k, c, base=base):
                rd(base + k, k).wait()
                compute(base + k, k)
                return c
            lax.fori_loop(0, n - 1, body, 0)
            rd(base + n - 1, n - 1).wait()

            def wbody(k, c, base=base):
                start_write(base + k, k)
                return c
            lax.fori_loop(0, n - 1, wbody, 0)
            compute(base + n - 1, n - 1)
            start_write(base + n - 1, n - 1)

            def wwbody(k, c, base=base):
                wait_write(base + k, k)
                return c
            lax.fori_loop(0, n, wwbody, 0)
            base += n
            if p + 1 < len(chunks):
                start_reads(base, chunks[p + 1])

    vmem_bytes = nslot * M * W * H * 2 + (8 << 20)
    xt = jnp.transpose(x, (0, 1, 3, 2)).reshape(G, M, J, R, S8, H)
    out = pl.pallas_call(
        kernel,
        in_specs=[pl.BlockSpec(memory_space=pltpu.SMEM),
                  pl.BlockSpec(memory_space=pltpu.SMEM),
                  pl.BlockSpec(memory_space=pl.ANY)],
        out_specs=pl.BlockSpec(memory_space=pl.ANY),
        out_shape=jax.ShapeDtypeStruct(xt.shape, x.dtype),
        scratch_shapes=[pltpu.VMEM((nslot, M, R, S8, H), jnp.bfloat16),
                        pltpu.VMEM((M, 8, 128), jnp.float32),
                        pltpu.VMEM((M, 8, 128), jnp.float32),
                        pltpu.SemaphoreType.DMA((nslot,)),
                        pltpu.SemaphoreType.DMA((nslot,))],
        compiler_params=pltpu.CompilerParams(vmem_limit_bytes=vmem_bytes),
    )(g.astype(jnp.float32), b.astype(jnp.float32), xt)
    return jnp.transpose(out.reshape(B, C, W, H), (0, 1, 3, 2))
```

```python
import jax
import jax.numpy as jnp
from jax import lax
import jax.experimental.pallas as pl
import jax.experimental.pallas.tpu as pltpu

_EPS = 1e-5


@jax.jit
def pallas_standalone__instancenorm__prompt_kernel(
    x: jax.Array,
    g: jax.Array,
    b: jax.Array,
):
    B, C, H, W = x.shape
    N = B * C
    S8 = 8
    R = W // S8
    M, J = 16, 8
    assert M * J == 128 and C % 128 == 0 and N % (M * J) == 0
    G = N // (M * J)
    nsub = G * J
    lgJ = J.bit_length() - 1
    nchunk = 3
    base_n = nsub // nchunk
    extra = nsub - base_n * nchunk
    nslot = base_n + extra
    inv_n = 1.0 / (H * W)
    RL = R - 1
    LA = 2
    LR = 4
    WQ = 4
    WR = 8
    SEG = M // RL
    NACC = 4
    CROWS = C // 128

    def kernel(g_hbm, b_hbm, x_hbm, o_hbm, buf, acc1, acc2, mu_ref, rs_ref,
               gb16, gb32, gbs, lsem, hsem, wsem, gsem):
        def gj(sub):
            return sub >> lgJ, sub & (J - 1)

        def l_copy(sub, slot, r):
            gi, j = gj(sub)
            return pltpu.make_async_copy(
                x_hbm.at[gi, :, j, r], buf.at[slot, :, r],
                lsem.at[(slot & (LR - 1)) * R + r])

        def h_copy(sub, slot, m):
            gi, j = gj(sub)
            return pltpu.make_async_copy(
                x_hbm.at[gi, m, j, RL], buf.at[slot, m, RL], hsem.at[0])

        def h_all(sub, slot):
            gi, j = gj(sub)
            return pltpu.make_async_copy(
                x_hbm.at[gi, :, j, RL], buf.at[slot, :, RL], hsem.at[0])

        def w_copy(sub, slot, r):
            gi, j = gj(sub)
            return pltpu.make_async_copy(
                buf.at[slot, :, r], o_hbm.at[gi, :, j, r],
                wsem.at[slot & (WR - 1)])

        def start_write(sub, slot):
            for r in range(R):
                w_copy(sub, slot, r).start()

        def wait_write(sub, slot):
            for r in range(R):
                w_copy(sub, slot, r).wait()

        def prime_reads(base):
            h_all(base, 0).start(priority=0)
            for s in range(LA + 1):
                for r in range(RL):
                    l_copy(base + s, s, r).start(priority=1)

        def tree(vals):
            while len(vals) > 1:
                vals = [vals[i] + vals[i + 1] for i in range(0, len(vals), 2)]
            return vals[0]

        def allreduce(a):
            a = jnp.sum(a, axis=2, keepdims=True)
            return jnp.sum(a, axis=1, keepdims=True)

        def lwait_refill(base, n, k, r):
            l_copy(base + k + 1, k + 1, r).wait()

            @pl.when(k + 2 + LA < n)
            def _():
                l_copy(base + k + 2 + LA, k + 2 + LA, r).start(priority=1)

        def step(base, n, k, do1, do2, do3, do_read):
            par = k & 1
            lo_off = 2 if do3 else (1 if do2 else 0)
            hi_off = 0 if do1 else (1 if do2 else 2)
            win = buf.at[pl.ds(k - lo_off, lo_off - hi_off + 1)]
            i1, i2, i3 = lo_off, lo_off - 1, lo_off - 2
            if do3:
                g3, j3 = gj(base + k - 2)
                row = lax.rem(g3, CROWS)

            def body(m, c):
                a1 = [None] * NACC
                a2 = [None] * NACC
                if do2:
                    mu2 = mu_ref[1 - par, m]
                kk = 0
                for r in range(R):
                    for q in range(H // 256):
                        cols = slice(q * 256, (q + 1) * 256)
                        if do1:
                            xf = win[i1, m, r, :, cols].astype(jnp.float32)
                        if do2:
                            yf = win[i2, m, r, :, cols].astype(jnp.float32)
                        for h in range(2):
                            i = kk % NACC
                            if do1:
                                v = xf[:, h * 128:(h + 1) * 128]
                                a1[i] = v if a1[i] is None else a1[i] + v
                            if do2:
                                d = yf[:, h * 128:(h + 1) * 128] - mu2
                                v = d * d
                                a2[i] = v if a2[i] is None else a2[i] + v
                            kk += 1
                if do3:
                    lane = m * J + j3
                    s = rs_ref[m] * gbs[0, row, lane]
                    t = gbs[1, row, lane] - mu_ref[par, m] * s
                    s2 = jnp.concatenate([s, s], axis=1)
                    t2 = jnp.concatenate([t, t], axis=1)
                    for r in range(R):
                        for q in range(H // 256):
                            cols = slice(q * 256, (q + 1) * 256)
                            zf = win[i3, m, r, :, cols].astype(jnp.float32)
                            win[i3, m, r, :, cols] = (zf * s2 + t2).astype(buf.dtype)
                if do1:
                    acc1[m] = tree(a1)
                if do2:
                    acc2[m] = tree(a2)
                if do_read:
                    h_copy(base + k + 1, k + 1, m).start(priority=0)
                return c

            if do_read:
                def seg(sg, c):
                    @pl.when(sg > 0)
                    def _():
                        lwait_refill(base, n, k, sg - 1)
                    lo = sg * SEG
                    hi = jnp.where(sg == RL - 1, M, lo + SEG)
                    lax.fori_loop(lo, hi, body, 0)
                    return c
                lax.fori_loop(0, RL, seg, 0)
            else:
                lax.fori_loop(0, M, body, 0)
            if do2:
                var = allreduce(acc2[...]) * inv_n
                rs_ref[...] = jnp.broadcast_to(lax.rsqrt(var + _EPS), (M, 8, 128))
            if do1:
                mu = allreduce(acc1[...]) * inv_n
                mu_ref[par] = jnp.broadcast_to(mu, (M, 8, 128))
            if do_read:
                lwait_refill(base, n, k, RL - 1)
                h_all(base + k + 1, k + 1).wait()

        prime_reads(0)
        gcp = pltpu.make_async_copy(g_hbm, gb16.at[0], gsem.at[0])
        bcp = pltpu.make_async_copy(b_hbm, gb16.at[1], gsem.at[1])
        gcp.start(priority=0)
        bcp.start(priority=0)
        gcp.wait()
        bcp.wait()
        gb32[...] = gb16[...].astype(jnp.float32)
        scp = pltpu.make_async_copy(gb32, gbs, gsem.at[0])
        scp.start()
        scp.wait()

        def chunk(p, c):
            n = jnp.where(p == 0, base_n + extra, base_n)
            base = jnp.where(p == 0, 0, p * base_n + extra)
            h_all(base, 0).wait()
            for r in range(RL):
                lwait_refill(base, n, -1, r)
            step(base, n, 0, True, False, False, True)
            step(base, n, 1, True, True, False, True)

            def main(k, c):
                step(base, n, k, True, True, True, True)
                return c
            lax.fori_loop(2, n - 1, main, 0)

            def w0(s, c):
                start_write(base + s, s)
                return c
            lax.fori_loop(0, WQ, w0, 0)
            step(base, n, n - 1, True, True, True, False)
            step(base, n, n, False, True, True, False)
            step(base, n, n + 1, False, False, True, False)

            def wloop(s, c):
                wait_write(base + s - WQ, s - WQ)
                start_write(base + s, s)
                return c
            lax.fori_loop(WQ, n, wloop, 0)

            def wtail(s, c):
                wait_write(base + s, s)
                return c
            lax.fori_loop(n - WQ, n, wtail, 0)

            @pl.when(p + 1 < nchunk)
            def _():
                prime_reads(base + n)
            return c
        lax.fori_loop(0, nchunk, chunk, 0)

    vmem_bytes = nslot * M * W * H * 2 + (8 << 20)
    xt = jnp.transpose(x, (0, 1, 3, 2)).reshape(G, M, J, R, S8, H)
    out = pl.pallas_call(
        kernel,
        in_specs=[pl.BlockSpec(memory_space=pl.ANY),
                  pl.BlockSpec(memory_space=pl.ANY),
                  pl.BlockSpec(memory_space=pl.ANY)],
        out_specs=pl.BlockSpec(memory_space=pl.ANY),
        out_shape=jax.ShapeDtypeStruct(xt.shape, x.dtype),
        scratch_shapes=[pltpu.VMEM((nslot, M, R, S8, H), x.dtype),
                        pltpu.VMEM((M, 8, 128), jnp.float32),
                        pltpu.VMEM((M, 8, 128), jnp.float32),
                        pltpu.VMEM((2, M, 8, 128), jnp.float32),
                        pltpu.VMEM((M, 8, 128), jnp.float32),
                        pltpu.VMEM((2, CROWS, 128), g.dtype),
                        pltpu.VMEM((2, CROWS, 128), jnp.float32),
                        pltpu.SMEM((2, CROWS, 128), jnp.float32),
                        pltpu.SemaphoreType.DMA((LR * R,)),
                        pltpu.SemaphoreType.DMA((1,)),
                        pltpu.SemaphoreType.DMA((WR,)),
                        pltpu.SemaphoreType.DMA((2,))],
        compiler_params=pltpu.CompilerParams(vmem_limit_bytes=vmem_bytes),
    )(g.reshape(CROWS, 128), b.reshape(CROWS, 128), xt)
    return jnp.transpose(out.reshape(B, C, W, H), (0, 1, 3, 2))
```

```python
import jax
import jax.numpy as jnp
from jax import lax
import jax.experimental.pallas as pl
import jax.experimental.pallas.tpu as pltpu

_EPS = 1e-5


@jax.jit
def pallas_standalone__instancenorm__prompt_kernel(
    x: jax.Array,
    g: jax.Array,
    b: jax.Array,
):
    B, C, H, W = x.shape
    N = B * C
    TR = 8
    ROWS = H * W // 128
    NT = ROWS // TR
    M, J = 16, 64
    G = N // (M * J)
    assert NT == 64 and N == G * M * J and C & (C - 1) == 0 and C % 128 == 0
    lgM = M.bit_length() - 1
    lgJ = J.bit_length() - 1
    NCHUNK = 3
    N0, N1 = 48, 40
    assert N0 + (NCHUNK - 1) * N1 == G * J
    inv_n = 1.0 / (H * W)
    CROWS = C // 128
    NACC = 4

    HP = (13, 16)
    LSEGS = (((0, 13),), ((29, 16),), ((45, 16), (61, 3)))
    NS = len(LSEGS)
    SEGM = (0, 5, 10, M)
    SPS = NS + 1
    MA = 4
    LA = 1
    LR = 2
    D = 2
    WP = ((0, 9), (9, 14), (23, 14), (37, 14), (51, 13))
    WM = 8
    NH = M // WM
    RUN = 8
    lgNH = NH.bit_length() - 1
    lgRUN = RUN.bit_length() - 1
    UQ = 3
    UR = 4

    def rs(t0, nt):
        return pl.ds(t0 * TR, nt * TR)

    def kernel(g_hbm, b_hbm, x_hbm, o_hbm, buf, acc1, acc2, mu_ref, rs_ref,
               spin_ref, gb16, gb32, gbs, lsem, hsem, wsem):
        def gj(sub):
            return sub >> lgJ, sub & (J - 1)

        def l_copies(sub, slot, sg, head=True, tail=True):
            gi, j = gj(sub)
            sb = (slot & (LR - 1)) * SPS

            def mk(ms, piece, si):
                return pltpu.make_async_copy(
                    x_hbm.at[gi, ms, j, rs(*piece)],
                    buf.at[slot, ms, rs(*piece)], lsem.at[sb + si])

            if sg < NS - 1:
                return [mk(slice(None), p, sg) for p in LSEGS[sg]]
            out = []
            if head:
                out.append(mk(pl.ds(0, MA), LSEGS[sg][0], sg))
            if tail:
                out.append(mk(pl.ds(MA, M - MA), LSEGS[sg][0], NS))
                out.extend(mk(slice(None), p, NS) for p in LSEGS[sg][1:])
            return out

        def h_copy(sub, slot, ms):
            gi, j = gj(sub)
            return pltpu.make_async_copy(
                x_hbm.at[gi, ms, j, rs(*HP)], buf.at[slot, ms, rs(*HP)],
                hsem.at[slot & 1])

        def unit(base, u):
            h = (u >> lgRUN) & (NH - 1)
            slot = ((u >> (lgRUN + lgNH)) << lgRUN) + (u & (RUN - 1))
            gi, j = gj(base + slot)
            return slot, pl.ds(h * WM, WM), gi, j

        def start_unit(base, u):
            slot, ms, gi, j = unit(base, u)
            for p in WP:
                pltpu.make_async_copy(
                    buf.at[slot, ms, rs(*p)], o_hbm.at[gi, ms, j, rs(*p)],
                    wsem.at[u & (UR - 1)]).start()

        def wait_unit(base, u):
            slot, ms, gi, j = unit(base, u)
            pltpu.make_async_copy(
                buf.at[slot, ms], o_hbm.at[gi, ms, j],
                wsem.at[u & (UR - 1)]).wait()

        def prime_reads(base):
            h_copy(base, 0, pl.ds(0, D)).start(priority=0)
            for s in range(LA + 1):
                for sg in range(NS):
                    for cp in l_copies(base + s, s, sg):
                        cp.start(priority=1)

        def lwait_refill(base, n, k, sg):
            for cp in l_copies(base + k + 1, k + 1, sg):
                cp.wait()

            @pl.when(k + 2 + LA < n)
            def _():
                for cp in l_copies(base + k + 2 + LA, k + 2 + LA, sg):
                    cp.start(priority=1)

        def tree(vals):
            while len(vals) > 1:
                vals = [vals[i] + vals[i + 1] for i in range(0, len(vals), 2)]
            return vals[0]

        def allreduce(a):
            a = jnp.sum(a, axis=2, keepdims=True)
            return jnp.sum(a, axis=1, keepdims=True)

        def spin(iters):
            def body(_, c):
                spin_ref[...] = spin_ref[...] * 0.5 + 1.0
                return c
            lax.fori_loop(0, iters, body, 0)

        def step(base, n, k, do1, do2, do3, read, pad=0):
            par = k & 1
            lo_off = 2 if do3 else (1 if do2 else 0)
            hi_off = 0 if do1 else (1 if do2 else 2)
            if do1 or do2 or do3:
                win = buf.at[pl.ds(k - lo_off, lo_off - hi_off + 1)]
            i1, i2, i3 = lo_off, lo_off - 1, lo_off - 2
            if do3:
                g3, j3 = gj(base + k - 2)
                c0 = g3 * (M * J) + j3

            def body(m, c):
                a1 = [None] * NACC
                a2 = [None] * NACC
                if do2:
                    mu2 = mu_ref[1 - par, m]
                kk = 0
                for q in range(ROWS // 16):
                    rows = slice(q * 16, (q + 1) * 16)
                    if do1:
                        xf = win[i1, m, rows, :].astype(jnp.float32)
                    if do2:
                        yf = win[i2, m, rows, :].astype(jnp.float32)
                    for h in range(2):
                        i = kk % NACC
                        if do1:
                            v = xf[h * 8:(h + 1) * 8]
                            a1[i] = v if a1[i] is None else a1[i] + v
                        if do2:
                            d = yf[h * 8:(h + 1) * 8] - mu2
                            v = d * d
                            a2[i] = v if a2[i] is None else a2[i] + v
                        kk += 1
                if do3:
                    ch = (c0 + m * J) & (C - 1)
                    row = ch >> 7
                    lane = ch & 127
                    s = rs_ref[m] * gbs[0, row, lane]
                    t = gbs[1, row, lane] - mu_ref[par, m] * s
                    s2 = jnp.concatenate([s, s], axis=0)
                    t2 = jnp.concatenate([t, t], axis=0)
                    for q in range(ROWS // 16):
                        rows = slice(q * 16, (q + 1) * 16)
                        zf = win[i3, m, rows, :].astype(jnp.float32)
                        win[i3, m, rows, :] = (zf * s2 + t2).astype(buf.dtype)
                if do1:
                    acc1[m] = tree(a1)
                if do2:
                    acc2[m] = tree(a2)
                if read == "paced":
                    hs = k + 1 + ((m + D) >> lgM)
                    h_copy(base + hs, hs, (m + D) & (M - 1)).start(priority=0)
                elif read == "last":
                    @pl.when(m + D < M)
                    def _():
                        h_copy(base + k + 1, k + 1, m + D).start(priority=0)
                if pad:
                    spin(pad)
                return c

            if read == "paced":
                def seg(sg, c):
                    lo, hi = jnp.int32(SEGM[0]), jnp.int32(SEGM[1])
                    for s_ in range(1, NS):
                        @pl.when(sg == s_)
                        def _():
                            lwait_refill(base, n, k, s_ - 1)
                        lo = jnp.where(sg == s_, SEGM[s_], lo)
                        hi = jnp.where(sg == s_, SEGM[s_ + 1], hi)
                    lax.fori_loop(lo, hi, body, 0)
                    return c
                lax.fori_loop(0, NS, seg, 0)
            else:
                lax.fori_loop(0, M, body, 0)
            if do2:
                var = allreduce(acc2[...]) * inv_n
                rs_ref[...] = jnp.broadcast_to(lax.rsqrt(var + _EPS), (M, 8, 128))
            if do1:
                mu = allreduce(acc1[...]) * inv_n
                mu_ref[par] = jnp.broadcast_to(mu, (M, 8, 128))
            if read == "paced":
                lwait_refill(base, n, k, NS - 1)
                h_copy(base + k + 1, k + 1, slice(None)).wait()

        prime_reads(0)
        gcp = pltpu.make_async_copy(g_hbm, gb16.at[0], wsem.at[0])
        bcp = pltpu.make_async_copy(b_hbm, gb16.at[1], wsem.at[1])
        scp = pltpu.make_async_copy(gb32, gbs, wsem.at[2])
        gcp.start(priority=0)
        bcp.start(priority=0)
        spin_ref[...] = jnp.zeros_like(spin_ref)

        def chunk(p, c):
            n = jnp.where(p == 0, N0, N1)
            base = jnp.where(p == 0, 0, N0 + (p - 1) * N1)
            nu = n * NH

            step(base, n, -1, False, False, False, "paced", pad=12)

            @pl.when(p == 0)
            def _():
                gcp.wait()
                bcp.wait()
                gb32[...] = gb16[...].astype(jnp.float32)
                scp.start()

            step(base, n, 0, True, False, False, "paced", pad=9)

            @pl.when(p == 0)
            def _():
                scp.wait()

            step(base, n, 1, True, True, False, "paced", pad=4)

            def main(k, c):
                step(base, n, k, True, True, True, "paced")
                return c
            lax.fori_loop(2, n - 2, main, 0)
            step(base, n, n - 2, True, True, True, "last")
            for sg in range(NS):
                for cp in l_copies(base + n - 1, n - 1, sg, tail=False):
                    cp.wait()

            start_unit(base, jnp.int32(0))

            def w0(u, c):
                start_unit(base, u)
                return c
            lax.fori_loop(1, UQ, w0, 0)
            for cp in l_copies(base + n - 1, n - 1, NS - 1, head=False):
                cp.wait()
            h_copy(base + n - 1, n - 1, slice(None)).wait()

            def wloop(u, c):
                wait_unit(base, u - UQ)
                start_unit(base, u)
                return c
            step(base, n, n - 1, True, True, True, None)
            wloop(jnp.int32(UQ), 0)
            step(base, n, n, False, True, True, None)
            wloop(jnp.int32(UQ + 1), 0)
            step(base, n, n + 1, False, False, True, None)
            lax.fori_loop(UQ + 2, nu, wloop, 0)

            def wtail(u, c):
                wait_unit(base, u)
                return c
            lax.fori_loop(nu - UQ, nu, wtail, 0)

            @pl.when(p + 1 < NCHUNK)
            def _():
                prime_reads(base + n)
            return c
        lax.fori_loop(0, NCHUNK, chunk, 0)

    xt = jnp.transpose(x, (0, 1, 3, 2)).reshape(N, W // TR, TR, H // 128, 128)
    xt = jnp.transpose(xt, (0, 1, 3, 2, 4)).reshape(G, M, J, ROWS, 128)
    out = pl.pallas_call(
        kernel,
        in_specs=[pl.BlockSpec(memory_space=pl.ANY),
                  pl.BlockSpec(memory_space=pl.ANY),
                  pl.BlockSpec(memory_space=pl.ANY)],
        out_specs=pl.BlockSpec(memory_space=pl.ANY),
        out_shape=jax.ShapeDtypeStruct(xt.shape, x.dtype),
        scratch_shapes=[pltpu.VMEM((N0, M, ROWS, 128), x.dtype),
                        pltpu.VMEM((M, 8, 128), jnp.float32),
                        pltpu.VMEM((M, 8, 128), jnp.float32),
                        pltpu.VMEM((2, M, 8, 128), jnp.float32),
                        pltpu.VMEM((M, 8, 128), jnp.float32),
                        pltpu.VMEM((8, 128), jnp.float32),
                        pltpu.VMEM((2, CROWS, 128), g.dtype),
                        pltpu.VMEM((2, CROWS, 128), jnp.float32),
                        pltpu.SMEM((2, CROWS, 128), jnp.float32),
                        pltpu.SemaphoreType.DMA((LR * SPS,)),
                        pltpu.SemaphoreType.DMA((2,)),
                        pltpu.SemaphoreType.DMA((UR,))],
        compiler_params=pltpu.CompilerParams(
            vmem_limit_bytes=N0 * M * ROWS * 128 * 2 + (8 << 20)),
    )(g.reshape(CROWS, 128), b.reshape(CROWS, 128), xt)
    out = out.reshape(N, W // TR, H // 128, TR, 128)
    out = jnp.transpose(out, (0, 1, 3, 2, 4)).reshape(B, C, W, H)
    return jnp.transpose(out, (0, 1, 3, 2))
```
